```python
import os as _os
_os.environ.setdefault("JAX_PLATFORMS", "cpu")
import jax
import jax.numpy as jnp

def _softmax(x, axis=-1):
    return jax.nn.softmax(x, axis=axis)
def _gelu(x):
    return jax.nn.gelu(x, approximate=True)
def _silu(x):
    return jax.nn.silu(x)
def _sigmoid(x):
    return jax.nn.sigmoid(x)
def _layernorm(x, axis=-1, eps=1e-5):
    m = jnp.mean(x, axis=axis, keepdims=True)
    v = jnp.var(x, axis=axis, keepdims=True)
    return (x - m) / jnp.sqrt(v + eps)
def _scatter_add(tgt, idx, src, axis=0):
    return tgt.at[idx].add(src)
def _segment_sum(src, seg, n):
    return jax.ops.segment_sum(src, seg, n)
class _Rng:
    def __init__(self, key):
        self._k = key
    def _next(self):
        self._k, sub = jax.random.split(self._k)
        return sub
    def normal(self, shape):
        return jax.random.normal(self._next(), shape, dtype=jnp.bfloat16)
    def randint(self, lo, hi, shape):
        return jax.random.randint(self._next(), shape, lo, hi, dtype=jnp.int32)
    def uniform(self, shape, lo=0.0, hi=1.0):
        return jax.random.uniform(self._next(), shape, jnp.bfloat16, lo, hi)
    def permutation(self, n):
        return jax.random.permutation(self._next(), n)


kernel_name = 'sequential_preLN__sliding_block__dense_activation_relu__prompt'

def setup_inputs():
    _rng = _Rng(jax.random.key(int.from_bytes(__import__("os").urandom(4), "little")))
    _w = (lambda a: (lambda t: t.astype(jnp.bfloat16) if jnp.issubdtype(t.dtype, jnp.floating) else t)(jnp.asarray(a)))
    def _A_setup():
        B, S, D = 1, 2048, 640
        return {
            "x": _w((lambda *s: _rng.normal(s) * 0.05)(B, S, D)),
            "wqkv": _w((lambda *s: _rng.normal(s) * 0.05)(D, 3 * D)),
            "wo": _w((lambda *s: _rng.normal(s) * 0.05)(D, D)),
        }
    _A_in = _A_setup()

    def _B_setup():
        B, S, D, Dff = 1, 2048, 640, 1536
        return {
            "x": _w((lambda *s: _rng.normal(s) * 0.05)(B, S, D)),
            "w1": _w((lambda *s: _rng.normal(s) * 0.05)(D, Dff)),
            "w2": _w((lambda *s: _rng.normal(s) * 0.05)(Dff, D)),
        }
    _B_in = _B_setup()

    return {
        "A_x": _A_in["x"],
        "A_wqkv": _A_in["wqkv"],
        "A_wo": _A_in["wo"],
        "B_x": _B_in["x"],
        "B_w1": _B_in["w1"],
        "B_w2": _B_in["w2"],
    }

def reference(A_x, A_wqkv, A_wo, B_x, B_w1, B_w2):
    def _A_ref(x, wqkv, wo):
        B, S, D = x.shape
        H = 32; Dh = D // H; W = 256
        qkv = (lambda x, *d: x.transpose(*d))((x @ wqkv).reshape(B, S, 3, H, Dh), 2, 0, 3, 1, 4)
        q, k, v = qkv[0], qkv[1], qkv[2]
        scores = jnp.einsum("bhqd,bhkd->bhqk", q, k) * (Dh ** -0.5)
        idx = jnp.arange(S)
        mask = (idx[:, None] - idx[None, :] >= 0) & (idx[:, None] - idx[None, :] < W)
        scores = jnp.where(mask[None, None], scores, -1e9)
        p = _softmax(scores, axis=-1)
        o = jnp.einsum("bhqk,bhkd->bhqd", p, v)
        return (lambda x, *d: x.transpose(*d))(o, 0, 2, 1, 3).reshape(B, S, D) @ wo

    def _B_ref(x, w1, w2):
        h = jnp.einsum("bsd,df->bsf", x, w1)
        zero = jnp.zeros_like(h)
        h = jnp.maximum(h, zero)
        return jnp.einsum("bsf,fd->bsd", h, w2)

    x = A_x
    h = x + _A_ref(_layernorm(x, axis=-1), A_wqkv, A_wo)
    h2 = h + _B_ref(_layernorm(h, axis=-1), B_w1, B_w2)
    return h2
```

```python
import functools, math
import jax
import jax.numpy as jnp
from jax import lax
import jax.experimental.pallas as pl
import jax.experimental.pallas.tpu as pltpu

S = 2048; D = 640; H = 32; DH = 20; W = 256; DFF = 1536
TT = 128
NTILE = S // TT
EPS = 1e-5
NT = (((1,), (1,)), ((), ()))
bf16 = jnp.bfloat16; f32 = jnp.float32; u32 = jnp.uint32
QSCALE = (DH ** -0.5) * math.log2(math.e)
L_LO = 2.0 ** -50
L_HI = 2.0 ** 100
O_BIG = 1e30

def as_u32(x): return pltpu.bitcast(x, u32)
def as_bf(x): return pltpu.bitcast(x, bf16)

def layernorm(x):
    m = jnp.mean(x, axis=-1, keepdims=True)
    xc = x - m
    v = jnp.mean(xc * xc, axis=-1, keepdims=True)
    return xc * lax.rsqrt(v + EPS)

def quads(y):
    rows = y.shape[0]
    lane = lax.broadcasted_iota(jnp.int32, (rows, 128), 1)
    out = []
    for g in range(8):
        c0 = (80 * g) // 128; c1 = (80 * g + 79) // 128
        a = y[:, 128 * c0:128 * c0 + 128]
        if c1 != c0:
            a = jnp.where(lane >= (80 * g) % 128, a, y[:, 128 * c1:128 * c1 + 128])
        out.append(a)
    return out

def fill_tables(tab):
    lane16 = lax.broadcasted_iota(jnp.int32, (16, 128), 1)
    row16 = lax.broadcasted_iota(jnp.int32, (16, 128), 0)
    ones = jnp.uint32(0xFFFFFFFF); zero = jnp.uint32(0)
    for h in range(32):
        lo = (20 * h) % 128
        tab[h] = jnp.where(((lane16 - lo) & 127) < 20, ones, zero)
    i = lane16 & 31
    lo = jnp.where(2 * row16 <= i, jnp.uint32(0xFFFF), zero)
    hi = jnp.where(2 * row16 + 1 <= i, jnp.uint32(0xFFFF0000), zero)
    tab[32] = lo | hi
    tab[33] = ~(lo | hi)

def make_consts():
    row32 = lax.broadcasted_iota(jnp.int32, (32, 128), 0)
    lane32 = lax.broadcasted_iota(jnp.int32, (32, 128), 1)
    tri_sel = row32 <= (lane32 & 31)
    blk = lax.broadcasted_iota(jnp.int32, (16, 128), 1) >> 5
    sub8 = lax.broadcasted_iota(jnp.int32, (8, 128), 0) < 4
    blkf = lane32 >> 5
    torder = [[0, 8, 1, 2, 3, 4, 5, 6, 7], [0, 8, 1, 2, 3, 4, 5, 6, 7], [0, 8, 7, 1, 2, 3, 4, 5, 6], [0, 8, 6, 7, 1, 2, 3, 4, 5]]
    torder[1] = [0, 8, 1] + [2, 3, 4, 5, 6, 7]
    torder[0] = [0, 8, 1, 2] + [4, 5, 6, 7, 3]
    torder = [[0, 8, 1, 2, 4, 5, 6, 7, 3], [0, 8, 1, 2, 3, 4, 5, 6, 7], [0, 8, 7, 1, 2, 3, 4, 5, 6], [0, 8, 6, 7, 1, 2, 3, 4, 5]]
    return dict(b0f=(blkf & 1) == 1, b1f=(blkf & 2) == 2, torder=torder, tri_sel=tri_sel, b0=(blk & 1) == 1, b1=(blk & 2) == 2, sub8=sub8)

def barrel(get, C, g0=0):
    z = jnp.zeros((16, 128), u32)
    def sel(c, x, y):
        if x is None and y is None: return None
        return jnp.where(c, z if x is None else x, z if y is None else y)
    dest = [[] for _ in range(4)]
    for gm in range(g0, 12):
        src = [get(s, gm - s) if 0 <= gm - s <= 8 else None for s in range(4)]
        t = [sel(C['b0'], src[(i + 1) % 4], src[i]) for i in range(4)]
        for i in range(4):
            d = sel(C['b1'], t[(i + 2) % 4], t[i])
            dest[i].append(z if d is None else d)
    return [as_bf(jnp.concatenate(dest[(-a) % 4], axis=0)) for a in range(4)]

def qk_exp(kq, qu, hm, C, tab, true_max=False, g0=0):
    tri = C['tri_sel']
    G = []
    for s in range(4):
        qs = qu[16 * s:16 * s + 16]
        parts = [qs & hm[(p - s) % 4] for p in range(4)]
        wT = as_bf(jnp.concatenate(parts, axis=0))
        order = [t for t in C['torder'][s] if s + t >= g0]
        lhs = jnp.concatenate([kq[16 * (s + t - g0):16 * (s + t - g0) + 16] for t in order], axis=0)
        st = lax.dot_general(as_bf(lhs), wT, NT, preferred_element_type=f32)
        gr = {t: st[32 * i:32 * i + 32] for i, t in enumerate(order)}
        if g0:
            out = {8: as_u32(jnp.exp2(jnp.where(tri, gr[8], -1e9)).astype(bf16))}
            for t in order[1:]: out[t] = as_u32(jnp.exp2(gr[t]).astype(bf16))
            G.append(out)
            continue
        comb = jnp.where(tri, gr[8], gr[0])
        if true_max:
            m = jnp.maximum(jnp.max(comb, axis=0, keepdims=True), jnp.max(st[64:288], axis=0, keepdims=True))
            comb = comb - m
            gr = {t: v - m for t, v in gr.items()}
        e = as_u32(jnp.exp2(comb).astype(bf16))
        out = {0: e & tab[33], 8: e & tab[32]}
        for t in range(1, 8): out[t] = as_u32(jnp.exp2(gr[t]).astype(bf16))
        G.append(out)
    return barrel(lambda s, t: G[s][t], C, g0)

def pv(P, vt3, C, bad):
    o = []
    for a in range(4):
        oa = jnp.dot(vt3(a), P[a], preferred_element_type=f32)
        l = oa[24:32]
        r = pl.reciprocal(l, approx=True)
        o3 = oa[0:24] * jnp.concatenate([r, r, r], axis=0)
        if bad is not None:
            t = o3[0:8] + o3[8:16] + o3[16:24]
            ok = (l >= L_LO) & (l <= L_HI) & (jnp.abs(t) <= O_BIG)
            bad = jnp.where(ok, bad, 1.0)
        if a:
            o3 = pltpu.roll(o3, 128 - 32 * a, 1)
        o.append(o3)
    rows = []
    for m in range(2):
        e, od = o[2 * m], o[2 * m + 1]
        rows += [e[0:16], jnp.where(C['sub8'], e[16:24], od[16:24]), od[0:16]]
    return jnp.concatenate(rows, axis=0), bad


def kernel(x_hbm, wqkv_hbm, wo_hbm, w1_hbm, w2_hbm, out_hbm,
           x_s, wq_s, wk_s, wv_s, wo_s, w1_s, w2_s, wvt_s, k_scr, vt_scr, q_all, ot_all, out_s, tab,
           h0, h1_, hid_s, in_sems, out_sems, *, CFG):
    NSUB = 2; LAG = 3; NPRE = 4
    NIT = (NTILE - 1 - LAG) // NSUB
    C = {}
    h_s = (h0, h1_)
    DEPTH = CFG.get('depth', 1)

    cp = pltpu.make_async_copy
    c_x0 = cp(x_hbm.at[0:2 * TT], x_s.at[0:2 * TT], in_sems.at[0])
    c_wk = cp(wqkv_hbm.at[:, D:2 * D], wk_s, in_sems.at[1])
    c_wq = cp(wqkv_hbm.at[:, 0:D], wq_s, in_sems.at[2])
    c_x1 = cp(x_hbm.at[2 * TT:4 * TT], x_s.at[2 * TT:4 * TT], in_sems.at[3])
    c_wv = cp(wqkv_hbm.at[:, 2 * D:3 * D], wv_s, in_sems.at[4])
    c_wo = cp(wo_hbm, wo_s, in_sems.at[5])
    c_w1 = cp(w1_hbm, w1_s, in_sems.at[6])
    c_w2 = cp(w2_hbm, w2_s, in_sems.at[7])
    def c_xi(it):
        r = pl.ds((4 + 2 * it) * TT, 2 * TT) if isinstance(it, int) else pl.ds(pl.multiple_of((4 + 2 * it) * TT, TT), 2 * TT)
        return cp(x_hbm.at[r], x_s.at[r], in_sems.at[8 + it])
    for c in [c_x0, c_wk, c_wq, c_x1, c_wv, c_wo, c_w1, c_xi(0), c_w2] + [c_xi(i) for i in range(1, NIT)]:
        c.start()

    fill_tables(tab)

    state = dict(bad=jnp.zeros((8, 128), f32))

    def rows(n, mult=TT):
        if isinstance(n, int): return pl.ds(n * mult, mult)
        return pl.ds(pl.multiple_of(n * mult, mult), mult)

    def t_pre(n):
        st = {}
        def fl():
            st['xn'] = layernorm(x_s[rows(n), :].astype(f32)).astype(bf16)
        def fq():
            q = jnp.dot(st['xn'], wq_s[...], preferred_element_type=f32) * QSCALE
            for g, t in enumerate(quads(q)):
                q_all[n, g] = t.astype(bf16)
        def fk():
            k = jnp.dot(st['xn'], wk_s[...], preferred_element_type=f32)
            for g, t in enumerate(quads(k)):
                k_scr[g, rows(n + 2, 64), :] = as_u32(t.astype(bf16))
        def fv(c):
            def f():
                vt = lax.dot_general(wvt_s[320 * c:320 * c + 320, :], st['xn'], NT, preferred_element_type=f32)
                ones = jnp.ones((8, 128), f32)
                rws = []
                for m in range(8):
                    v0 = vt[40 * m:40 * m + 16]; v2 = vt[40 * m + 16:40 * m + 24]; v3 = vt[40 * m + 24:40 * m + 40]
                    rws += [v0, v2, ones, v3, v2, ones]
                vt_scr[n + 2, 512 * c:512 * c + 512, :] = jnp.concatenate(rws, axis=0).astype(bf16)
            return f
        return dict(l=fl, k=fk, v0=fv(0), v1=fv(1), q=fq)

    PV_ = {}
    def do_qk(n, g, key, slow=False):
        t0 = max(2 - n, 0) if isinstance(n, int) else 0
        kr = pl.ds((n + t0) * 64, 192 - 64 * t0) if isinstance(n, int) else pl.ds(pl.multiple_of(n * 64, 64), 192)
        hm = [tab[4 * g + a] for a in range(4)]
        PV_[key] = qk_exp(k_scr[g, kr, :], as_u32(q_all[n, g]), hm, C, tab, slow, 4 * t0)
    def do_pv(n, g, key, slow=False):
        def vt3(a):
            t0 = max(2 - n, 0) if isinstance(n, int) else 0
            return jnp.concatenate([vt_scr[n + t, rows(4 * g + a, 32), :] for t in range(t0, 3)], axis=1)
        o, bad = pv(PV_.pop(key), vt3, C, None if slow or not CFG.get('check', True) else state['bad'])
        if bad is not None: state['bad'] = bad
        orow = pl.ds(80 * g, 80) if isinstance(g, int) else pl.ds(pl.multiple_of(80 * g, 16), 80)
        ot_all[n, orow, :] = o.astype(bf16)

    def stream(tiles, fill, tail=(), depth=DEPTH, started=0):
        sus = [(n, g, (i, g)) for i, n in enumerate(tiles) for g in range(8)]
        nq = started
        m = len(fill); nsu = len(sus); done = 0
        for i in range(nsu):
            while nq < min(i + depth + 1, nsu):
                do_qk(*sus[nq]); nq += 1
            want = (m * (i + 1) + nsu - 1) // nsu if m else 0
            while done < min(want, m):
                fill[done](); done += 1
            do_pv(*sus[i])
        for f in list(fill[done:]) + list(tail): f()

    NC = 3; cw = DFF // NC
    def t_post(n, slot):
        st = {}
        hs = h_s[slot]
        def fo():
            o = ot_all[n].astype(f32).T.astype(bf16)
            att = jnp.dot(o, wo_s[...], preferred_element_type=f32)
            h = x_s[rows(n), :].astype(f32) + att
            if CFG.get('hval', 0): st['h'] = h
            else: hs[...] = h
        def fl():
            st['hn'] = layernorm(st['h'] if CFG.get('hval', 0) else hs[...]).astype(bf16)
            st['h1'] = []
        def f1(c):
            def f():
                y = jnp.dot(st['hn'], w1_s[:, c * cw:(c + 1) * cw], preferred_element_type=f32)
                st['h1'].append(jnp.maximum(y, 0.0).astype(bf16))
            return f
        def f2(c, dma=None):
            def f():
                y = (st['h'] if CFG.get('hval', 0) else hs)[:, c * 128:(c + 1) * 128]
                for kc in range(NC):
                    y = y + jnp.dot(st['h1'][kc], w2_s[kc * cw:(kc + 1) * cw, c * 128:(c + 1) * 128], preferred_element_type=f32)
                out_s[rows(n), c * 128:(c + 1) * 128] = y.astype(bf16)
            return f
        return dict(o=fo, l=fl, f1=[f1(c) for c in range(NC)], f2=[f2(c) for c in range(5)])

    def out_copy(n, cnt, sem):
        r = pl.ds(n * TT, cnt * TT) if isinstance(n, int) else pl.ds(pl.multiple_of(n * TT, TT), cnt * TT)
        return cp(out_s.at[r], out_hbm.at[r], out_sems.at[sem])
    def last_copy(c):
        r = pl.ds((NTILE - 1) * TT, TT); cs = pl.ds(c * 128, 128)
        return cp(out_s.at[r, cs], out_hbm.at[r, cs], out_sems.at[NIT + 3 + c])

    C.update(make_consts())
    P = [t_pre(n) for n in range(NPRE)]
    c_x0.wait()
    P[0]['l'](); P[1]['l']()
    c_wk.wait()
    P[0]['k'](); P[1]['k']()
    c_wq.wait()
    P[0]['q'](); P[1]['q']()
    do_qk(0, 0, (0, 0)); do_qk(0, 1, (0, 1))
    c_x1.wait(); c_wv.wait()
    wvt_s[...] = wv_s[...].astype(f32).T.astype(bf16)
    P[2]['l'](); P[3]['l']()
    NA = CFG.get('na', 4)
    for g in range(2, NA): do_qk(0, g, (0, g))
    P[2]['k']()
    P[0]['v0'](); P[0]['v1']()
    fill = [P[1]['v0'], P[1]['v1'], P[2]['q'], P[2]['v0'], P[2]['v1'], P[3]['k'], P[3]['v0'], P[3]['v1'], P[3]['q']]
    nop = lambda: None
    fill = [fill[i] if i >= 0 else nop for i in CFG.get('pfill', [0, -1, 1, -1, 2, 3, 4, -1, 5, 6, -1, 7])]
    stream([0, 1, 2], fill, tail=[P[3]['q']], started=NA, depth=CFG.get('pdepth', 1))
    for c in (c_wo, c_w1, c_w2): c.wait()
    for it in range(CFG.get('nit', NIT), NIT): c_xi(it).wait()

    def tile_fill(n, slot):
        F = t_post(n - LAG, slot); Pn = t_pre(n + 1)
        return [Pn['l'], F['o'], Pn['k'], F['l'], Pn['v0'], Pn['v1']] + F['f1'] + [Pn['q']] + F['f2']

    NTAIL = CFG.get('ntail', 2)
    def loop_body(it, bad):
        state['bad'] = bad
        C.update(make_consts())
        n0 = LAG + it * NSUB
        c_xi(it).wait()
        fill = tile_fill(n0, 0) + tile_fill(n0 + 1, 1)
        stream([n0, n0 + 1], fill[:len(fill) - NTAIL], tail=fill[len(fill) - NTAIL:])
        out_copy(n0 - LAG, NSUB, it).start()
        return state['bad']

    state['bad'] = lax.fori_loop(0, CFG.get('nit', NIT), loop_body, state['bad'])

    C.update(make_consts())
    F = [t_post(NTILE - 4 + i, i % 2) for i in range(4)]
    st_ = lambda i: (lambda: out_copy(NTILE - 4 + i, 1, NIT + i).start())
    fill = [F[0]['o'], F[0]['l'], F[1]['o']] + F[0]['f1'] + [F[1]['l']] + F[0]['f2'] + [st_(0)]
    stream([NTILE - 1], fill)
    seq = F[1]['f1'] + [F[2]['o'], F[2]['l']] + F[1]['f2'] + [st_(1)] + F[2]['f1'] + [F[3]['o'], F[3]['l']] + F[2]['f2'] + [st_(2)] + F[3]['f1']
    for c in range(5):
        seq += [F[3]['f2'][c], functools.partial(lambda c: last_copy(c).start(), c)]
    for f in seq: f()

    for it in range(CFG.get('nit', NIT)):
        out_copy(it * NSUB, NSUB, it).wait()
    for i in range(3):
        out_copy(NTILE - 4 + i, 1, NIT + i).wait()
    for c in range(5):
        last_copy(c).wait()

    if CFG.get('fallback', True):
        flag = jnp.max(state['bad'])
        @pl.when(flag > 0.0)
        def _():
            vt_scr[0:2] = jnp.zeros((2,) + vt_scr.shape[1:], vt_scr.dtype)
            for g in range(8):
                w0 = k_scr[g, 128:129, :] & jnp.uint32(0xFFFF)
                k_scr[g, 0:128, :] = jnp.broadcast_to(w0 | (w0 << 16), (128, 128))
            def slow_tile(n, carry):
                C.update(make_consts())
                def slow_g(g, c2):
                    do_qk(n, g, 'slow', True); do_pv(n, g, 'slow', True)
                    return c2
                lax.fori_loop(0, 8, slow_g, 0)
                o = ot_all[n].astype(f32).T.astype(bf16)
                h0[...] = x_s[rows(n), :].astype(f32) + jnp.dot(o, wo_s[...], preferred_element_type=f32)
                hn = layernorm(h0[...]).astype(bf16)
                def s1(c, c2):
                    cs = pl.ds(pl.multiple_of(c * 128, 128), 128)
                    hid_s[:, cs] = jnp.maximum(jnp.dot(hn, w1_s[:, cs], preferred_element_type=f32), 0.0).astype(bf16)
                    return c2
                lax.fori_loop(0, DFF // 128, s1, 0)
                def s2(c, c2):
                    cs = pl.ds(pl.multiple_of(c * 128, 128), 128)
                    y = h0[:, cs] + jnp.dot(hid_s[...], w2_s[:, cs], preferred_element_type=f32)
                    out_s[rows(n), cs] = y.astype(bf16)
                    return c2
                lax.fori_loop(0, D // 128, s2, 0)
                return carry
            lax.fori_loop(0, NTILE, slow_tile, 0)
            c = cp(out_s, out_hbm, out_sems.at[0])
            c.start(); c.wait()


@jax.jit
def pallas_sequential_preLN__sliding_block__dense_activation_relu__prompt_kernel(
    A_x: jax.Array,
    A_wqkv: jax.Array,
    A_wo: jax.Array,
    B_x: jax.Array,
    B_w1: jax.Array,
    B_w2: jax.Array,
):
    V = pltpu.VMEM
    NIT = 6
    x = A_x.reshape(S, D)
    out = pl.pallas_call(
        functools.partial(kernel, CFG={'pdepth': 2}),
        in_specs=[pl.BlockSpec(memory_space=pl.ANY)] * 5,
        out_specs=pl.BlockSpec(memory_space=pl.ANY),
        out_shape=jax.ShapeDtypeStruct((S, D), bf16),
        scratch_shapes=[V((S, D), bf16), V((D, D), bf16), V((D, D), bf16), V((D, D), bf16), V((D, D), bf16),
                        V((D, DFF), bf16), V((DFF, D), bf16), V((D, D), bf16),
                        V((8, (S + W) // 2, 128), u32), V((NTILE + 2, 1024, 128), bf16),
                        V((NTILE, 8, TT, 128), bf16), V((NTILE, D, TT), bf16), V((S, D), bf16),
                        V((34, 16, 128), u32), V((TT, D), f32), V((TT, D), f32), V((TT, DFF), bf16),
                        pltpu.SemaphoreType.DMA((8 + NIT,)), pltpu.SemaphoreType.DMA((NIT + 8,))],
        compiler_params=pltpu.CompilerParams(vmem_limit_bytes=100 * 1024 * 1024),
    )(x, A_wqkv, A_wo, B_w1, B_w2)
    return out.reshape(1, S, D)
```

```python
import functools
import math

import jax
import jax.numpy as jnp
from jax import lax
import jax.experimental.pallas as pl
import jax.experimental.pallas.tpu as pltpu

S = 2048
D = 640
DH = 20
W = 256
DFF = 1536
TT = 128
NTILE = S // TT
NSUB = 2
LAG = 3
NIT = (NTILE - 1 - LAG) // NSUB
NC = 3
CW = DFF // NC
KA = 256
EPS = 1e-5
NT = (((1,), (1,)), ((), ()))
bf16 = jnp.bfloat16
f32 = jnp.float32
u32 = jnp.uint32
QSCALE = (DH ** -0.5) * math.log2(math.e)
L_LO = 2.0 ** -50
L_HI = 2.0 ** 100
O_BIG = 1e30
TORDER = ((0, 8, 1, 2, 4, 5, 6, 7, 3), (0, 8, 1, 2, 3, 4, 5, 6, 7),
          (0, 8, 7, 1, 2, 3, 4, 5, 6), (0, 8, 6, 7, 1, 2, 3, 4, 5))


def _as_u32(x):
    return pltpu.bitcast(x, u32)


def _as_bf(x):
    return pltpu.bitcast(x, bf16)


def _rows(n, size, count=1):
    if isinstance(n, int):
        return pl.ds(n * size, count * size)
    return pl.ds(pl.multiple_of(n * size, size), count * size)


def _layernorm(x):
    m = jnp.mean(x, axis=-1, keepdims=True)
    xc = x - m
    v = jnp.mean(xc * xc, axis=-1, keepdims=True)
    return xc * lax.rsqrt(v + EPS)


def _quads(y):
    lane = lax.broadcasted_iota(jnp.int32, (y.shape[0], 128), 1)
    out = []
    for g in range(8):
        c0 = (80 * g) // 128
        c1 = (80 * g + 79) // 128
        a = y[:, 128 * c0:128 * c0 + 128]
        if c1 != c0:
            a = jnp.where(lane >= (80 * g) % 128, a, y[:, 128 * c1:128 * c1 + 128])
        out.append(a)
    return out


def _fill_tables(tab):
    lane = lax.broadcasted_iota(jnp.int32, (16, 128), 1)
    row = lax.broadcasted_iota(jnp.int32, (16, 128), 0)
    ones = jnp.uint32(0xFFFFFFFF)
    zero = jnp.uint32(0)
    for h in range(32):
        tab[h] = jnp.where(((lane - (20 * h) % 128) & 127) < 20, ones, zero)
    i = lane & 31
    low = (jnp.where(2 * row <= i, jnp.uint32(0xFFFF), zero)
           | jnp.where(2 * row + 1 <= i, jnp.uint32(0xFFFF0000), zero))
    tab[32] = low
    tab[33] = ~low


def _masks():
    row32 = lax.broadcasted_iota(jnp.int32, (32, 128), 0)
    lane32 = lax.broadcasted_iota(jnp.int32, (32, 128), 1)
    blk = lax.broadcasted_iota(jnp.int32, (16, 128), 1) >> 5
    return dict(tri=row32 <= (lane32 & 31), b0=(blk & 1) == 1, b1=(blk & 2) == 2,
                sub8=lax.broadcasted_iota(jnp.int32, (8, 128), 0) < 4)


def _scores_to_probs(kq, qu, hm, M, tab, true_max, g0):
    tri = M['tri']
    probs = []
    for s in range(4):
        qs = qu[16 * s:16 * s + 16]
        w_t = _as_bf(jnp.concatenate([qs & hm[(p - s) % 4] for p in range(4)], axis=0))
        order = [t for t in TORDER[s] if s + t >= g0]
        lhs = jnp.concatenate([kq[16 * (s + t - g0):16 * (s + t - g0) + 16] for t in order], axis=0)
        st = lax.dot_general(_as_bf(lhs), w_t, NT, preferred_element_type=f32)
        gr = {t: st[32 * i:32 * i + 32] for i, t in enumerate(order)}
        if g0:
            out = {8: _as_u32(jnp.exp2(jnp.where(tri, gr[8], -1e9)).astype(bf16))}
            rest = order[1:]
        else:
            comb = jnp.where(tri, gr[8], gr[0])
            if true_max:
                m = jnp.maximum(jnp.max(comb, axis=0, keepdims=True),
                                jnp.max(st[64:], axis=0, keepdims=True))
                comb = comb - m
                gr = {t: v - m for t, v in gr.items()}
            e = _as_u32(jnp.exp2(comb).astype(bf16))
            out = {0: e & tab[33], 8: e & tab[32]}
            rest = order[2:]
        for t in rest:
            out[t] = _as_u32(jnp.exp2(gr[t]).astype(bf16))
        probs.append(out)

    z = jnp.zeros((16, 128), u32)

    def sel(c, x, y):
        if x is None and y is None:
            return None
        return jnp.where(c, z if x is None else x, z if y is None else y)

    dest = [[] for _ in range(4)]
    for gm in range(g0, 12):
        src = [probs[s].get(gm - s) for s in range(4)]
        t = [sel(M['b0'], src[(i + 1) % 4], src[i]) for i in range(4)]
        for i in range(4):
            d = sel(M['b1'], t[(i + 2) % 4], t[i])
            dest[i].append(z if d is None else d)
    return [_as_bf(jnp.concatenate(dest[(-a) % 4], axis=0)) for a in range(4)]


def _probs_to_out(P, vt, M, bad):
    o = []
    for a in range(4):
        oa = jnp.dot(vt(a), P[a], preferred_element_type=f32)
        l = oa[24:32]
        r = pl.reciprocal(l, approx=True)
        o3 = oa[0:24] * jnp.concatenate([r, r, r], axis=0)
        if bad is not None:
            t = o3[0:8] + o3[8:16] + o3[16:24]
            ok = (l >= L_LO) & (l <= L_HI) & (jnp.abs(t) <= O_BIG)
            bad = jnp.where(ok, bad, 1.0)
        if a:
            o3 = pltpu.roll(o3, 128 - 32 * a, 1)
        o.append(o3)
    rows = []
    for m in range(2):
        e, od = o[2 * m], o[2 * m + 1]
        rows += [e[0:16], jnp.where(M['sub8'], e[16:24], od[16:24]), od[0:16]]
    return jnp.concatenate(rows, axis=0), bad


def _kernel(x_hbm, wqkv_hbm, wo_hbm, w1_hbm, w2_hbm, out_hbm,
            x_s, wq_s, wk_s, wv_s, wo_s, w1_s, w2_s, wvt_s, k_s, vt_s, q_s, o_s, out_s, tab,
            ot0, ot1, h0, h1, hid_s, in_sems, out_sems):
    cp = pltpu.make_async_copy
    ot_s = (ot0, ot1)
    h_s = (h0, h1)
    M = {}
    state = dict(bad=jnp.zeros((8, 128), f32))

    def x_copy(n, count, sem):
        r = _rows(n, TT, count)
        return cp(x_hbm.at[r], x_s.at[r], in_sems.at[sem])

    c_x0 = x_copy(0, 3, 0)
    c_wka = cp(wqkv_hbm.at[:, D:D + KA], wk_s.at[:, 0:KA], in_sems.at[1])
    c_wkb = cp(wqkv_hbm.at[:, D + KA:2 * D], wk_s.at[:, KA:D], in_sems.at[2])
    c_wq = cp(wqkv_hbm.at[:, 0:D], wq_s, in_sems.at[3])
    c_x1 = x_copy(3, 1, 4)
    c_wv = cp(wqkv_hbm.at[:, 2 * D:3 * D], wv_s, in_sems.at[5])
    c_wo = cp(wo_hbm, wo_s, in_sems.at[6])
    c_w1 = cp(w1_hbm, w1_s, in_sems.at[7])
    c_w2 = cp(w2_hbm, w2_s, in_sems.at[8])

    def c_xi(it):
        return x_copy(LAG + 1 + NSUB * it, NSUB, 9 + it)

    for c in [c_x0, c_wka, c_wkb, c_wq, c_x1, c_wv, c_wo, c_w1, c_xi(0), c_w2]:
        c.start()
    for it in range(1, NIT):
        c_xi(it).start()

    _fill_tables(tab)

    def pre_tasks(n):
        st = {}

        def put_k(k):
            for g, t in enumerate(_quads(k)):
                k_s[g, _rows(n + 2, 64), :] = _as_u32(t.astype(bf16))

        def ln():
            st['xn'] = _layernorm(x_s[_rows(n, TT), :].astype(f32)).astype(bf16)

        def q():
            y = jnp.dot(st['xn'], wq_s[...], preferred_element_type=f32) * QSCALE
            for g, t in enumerate(_quads(y)):
                q_s[n, g] = t.astype(bf16)

        def k():
            put_k(jnp.dot(st['xn'], wk_s[...], preferred_element_type=f32))

        def ka():
            st['ka'] = jnp.dot(st['xn'], wk_s[:, 0:KA], preferred_element_type=f32)

        def kb():
            y = jnp.dot(st['xn'], wk_s[:, KA:D], preferred_element_type=f32)
            put_k(jnp.concatenate([st['ka'], y], axis=1))

        def v(c):
            vt = lax.dot_general(wvt_s[320 * c:320 * c + 320, :], st['xn'], NT, preferred_element_type=f32)
            ones = jnp.ones((8, 128), f32)
            rows = []
            for m in range(8):
                mid = vt[40 * m + 16:40 * m + 24]
                rows += [vt[40 * m:40 * m + 16], mid, ones, vt[40 * m + 24:40 * m + 40], mid, ones]
            vt_s[n + 2, 512 * c:512 * c + 512, :] = jnp.concatenate(rows, axis=0).astype(bf16)

        return dict(ln=ln, q=q, k=k, ka=ka, kb=kb, v0=lambda: v(0), v1=lambda: v(1))

    pending = {}

    def do_qk(n, g, key, slow=False):
        t0 = max(2 - n, 0) if isinstance(n, int) else 0
        hm = [tab[4 * g + a] for a in range(4)]
        pending[key] = _scores_to_probs(k_s[g, _rows(n + t0, 64, 3 - t0), :], _as_u32(q_s[n, g]),
                                        hm, M, tab, slow, 4 * t0)

    def do_pv(n, g, key, par, slow=False):
        t0 = max(2 - n, 0) if isinstance(n, int) else 0

        def vt(a):
            return jnp.concatenate([vt_s[n + t, _rows(4 * g + a, 32), :] for t in range(t0, 3)], axis=1)

        o, bad = _probs_to_out(pending.pop(key), vt, M, None if slow else state['bad'])
        if not slow:
            state['bad'] = bad
        ot_s[par][_rows(5 * g, 16, 5), :] = o.astype(bf16)

    def transpose_task(n, par):
        def f():
            o_s[n] = ot_s[par][...].astype(f32).T.astype(bf16)
        return f

    def attention(tiles, par0, fill, head=(), tail=(), depth=1, started=0):
        units = [(n, g, (i, g)) for i, n in enumerate(tiles) for g in range(8)]
        nq, done = started, 0
        for f in head:
            f()
        for i, u in enumerate(units):
            while nq < min(i + depth + 1, len(units)):
                do_qk(*units[nq])
                nq += 1
            while done < -(-len(fill) * (i + 1) // len(units)):
                fill[done]()
                done += 1
            do_pv(*u, par=(par0 + i // 8) % 2)
        for f in tail:
            f()

    def post_tasks(n, slot):
        st = {'h1': []}
        hs = h_s[slot]

        def proj():
            att = jnp.dot(o_s[n], wo_s[...], preferred_element_type=f32)
            hs[...] = x_s[_rows(n, TT), :].astype(f32) + att

        def ln():
            st['hn'] = _layernorm(hs[...]).astype(bf16)

        def up(c):
            y = jnp.dot(st['hn'], w1_s[:, c * CW:(c + 1) * CW], preferred_element_type=f32)
            st['h1'].append(jnp.maximum(y, 0.0).astype(bf16))

        def down(c):
            cs = slice(c * 128, (c + 1) * 128)
            y = hs[:, cs]
            for kc in range(NC):
                y = y + jnp.dot(st['h1'][kc], w2_s[kc * CW:(kc + 1) * CW, cs], preferred_element_type=f32)
            out_s[_rows(n, TT), cs] = y.astype(bf16)

        return dict(proj=proj, ln=ln, up=[functools.partial(up, c) for c in range(NC)],
                    down=[functools.partial(down, c) for c in range(D // 128)])

    def out_copy(n, count, sem):
        r = _rows(n, TT, count)
        return cp(out_s.at[r], out_hbm.at[r], out_sems.at[sem])

    def last_copy(c):
        r = _rows(NTILE - 1, TT)
        cs = pl.ds(c * 128, 128)
        return cp(out_s.at[r, cs], out_hbm.at[r, cs], out_sems.at[NIT + LAG + c])

    M.update(_masks())
    P = [pre_tasks(n) for n in range(LAG + 1)]
    c_x0.wait()
    P[0]['ln']()
    P[1]['ln']()
    c_wka.wait()
    P[2]['ln']()
    for n in range(3):
        P[n]['ka']()
    c_wkb.wait()
    for n in range(3):
        P[n]['kb']()
    c_wq.wait()
    P[0]['q']()
    P[1]['q']()
    for g in range(8):
        do_qk(0, g, (0, g))
    c_x1.wait()
    c_wv.wait()
    wvt_s[...] = wv_s[...].astype(f32).T.astype(bf16)
    P[3]['ln']()
    P[2]['q']()
    P[0]['v0']()
    P[0]['v1']()

    def nop():
        pass

    fill = [P[1]['v0'], nop, P[1]['v1'], nop, nop, transpose_task(0, 0), P[2]['v0'], P[2]['v1'], nop,
            P[3]['k'], transpose_task(1, 1), P[3]['v0'], P[3]['v1']]
    attention([0, 1, 2], 0, fill, tail=[P[3]['q']], depth=3, started=8)
    c_wo.wait()
    c_w1.wait()
    c_w2.wait()

    def tile_fill(n, par):
        F = post_tasks(n - LAG, par)
        N = pre_tasks(n + 1)
        return ([F['proj'], N['ln'], N['k'], F['ln'], transpose_task(n - 1, par), N['v0'], N['v1'], N['q']]
                + F['up'] + F['down'])

    def loop_body(it, bad):
        state['bad'] = bad
        M.update(_masks())
        n0 = LAG + it * NSUB
        c_xi(it).wait()
        fill = tile_fill(n0, 0) + tile_fill(n0 + 1, 1)
        attention([n0, n0 + 1], 1, fill[1:-1], head=fill[:1], tail=fill[-1:])
        out_copy(n0 - LAG, NSUB, it).start()
        return state['bad']

    state['bad'] = lax.fori_loop(0, NIT, loop_body, state['bad'])

    M.update(_masks())
    n0 = NTILE - 1 - LAG
    F = [post_tasks(n0 + i, i % 2) for i in range(LAG + 1)]

    def send(i):
        return lambda: out_copy(n0 + i, 1, NIT + i).start()

    fill = ([transpose_task(NTILE - 2, 0), F[0]['ln'], F[1]['proj']] + F[0]['up'] + [F[1]['ln']]
            + F[0]['down'] + [send(0)])
    attention([NTILE - 1], 1, fill, head=[F[0]['proj']])
    unsafe = jnp.max(state['bad'])
    seq = [transpose_task(NTILE - 1, 1)]
    for i in range(1, LAG):
        seq += F[i]['up'] + [F[i + 1]['proj'], F[i + 1]['ln']] + F[i]['down'] + [send(i)]
    seq += F[LAG]['up']
    for f in seq:
        f()
    for c in range(D // 128):
        F[LAG]['down'][c]()
        last_copy(c).start()

    for it in range(NIT):
        out_copy(it * NSUB, NSUB, it).wait()
    for i in range(LAG):
        out_copy(n0 + i, 1, NIT + i).wait()
    for c in range(D // 128):
        last_copy(c).wait()

    @pl.when(unsafe > 0.0)
    def _():
        vt_s[0:2] = jnp.zeros((2,) + vt_s.shape[1:], bf16)
        for g in range(8):
            k0 = k_s[g, 128:129, :] & jnp.uint32(0xFFFF)
            k_s[g, 0:128, :] = jnp.broadcast_to(k0 | (k0 << 16), (128, 128))

        def slow_tile(n, carry):
            M.update(_masks())

            def slow_quad(g, c):
                do_qk(n, g, 'slow', True)
                do_pv(n, g, 'slow', 0, True)
                return c

            lax.fori_loop(0, 8, slow_quad, 0)
            o = ot0[...].astype(f32).T.astype(bf16)
            h0[...] = x_s[_rows(n, TT), :].astype(f32) + jnp.dot(o, wo_s[...], preferred_element_type=f32)
            hn = _layernorm(h0[...]).astype(bf16)

            def slow_up(c, c2):
                cs = _rows(c, 128)
                y = jnp.dot(hn, w1_s[:, cs], preferred_element_type=f32)
                hid_s[:, cs] = jnp.maximum(y, 0.0).astype(bf16)
                return c2

            lax.fori_loop(0, DFF // 128, slow_up, 0)

            def slow_down(c, c2):
                cs = _rows(c, 128)
                y = h0[:, cs] + jnp.dot(hid_s[...], w2_s[:, cs], preferred_element_type=f32)
                out_s[_rows(n, TT), cs] = y.astype(bf16)
                return c2

            lax.fori_loop(0, D // 128, slow_down, 0)
            return carry

        lax.fori_loop(0, NTILE, slow_tile, 0)
        c = cp(out_s, out_hbm, out_sems.at[0])
        c.start()
        c.wait()


@jax.jit
def pallas_sequential_preLN__sliding_block__dense_activation_relu__prompt_kernel(
    A_x: jax.Array,
    A_wqkv: jax.Array,
    A_wo: jax.Array,
    B_x: jax.Array,
    B_w1: jax.Array,
    B_w2: jax.Array,
):
    del B_x
    V = pltpu.VMEM
    hbm = pl.BlockSpec(memory_space=pl.ANY)
    out = pl.pallas_call(
        _kernel,
        in_specs=[hbm] * 5,
        out_specs=hbm,
        out_shape=jax.ShapeDtypeStruct((S, D), bf16),
        scratch_shapes=[
            V((S, D), bf16),
            V((D, D), bf16), V((D, D), bf16), V((D, D), bf16), V((D, D), bf16),
            V((D, DFF), bf16), V((DFF, D), bf16),
            V((D, D), bf16),
            V((8, (S + W) // 2, 128), u32),
            V((NTILE + 2, 1024, 128), bf16),
            V((NTILE, 8, TT, 128), bf16),
            V((NTILE, TT, D), bf16),
            V((S, D), bf16),
            V((34, 16, 128), u32),
            V((D, TT), bf16), V((D, TT), bf16),
            V((TT, D), f32), V((TT, D), f32),
            V((TT, DFF), bf16),
            pltpu.SemaphoreType.DMA((9 + NIT,)),
            pltpu.SemaphoreType.DMA((NIT + LAG + D // 128,)),
        ],
        compiler_params=pltpu.CompilerParams(vmem_limit_bytes=100 * 1024 * 1024),
    )(A_x.reshape(S, D), A_wqkv, A_wo, B_w1, B_w2)
    return out.reshape(1, S, D)
```

```python
import functools
import math

import jax
import jax.numpy as jnp
from jax import lax
import jax.experimental.pallas as pl
import jax.experimental.pallas.tpu as pltpu

S = 2048
D = 640
DH = 20
W = 256
DFF = 1536
TT = 128
NTILE = S // TT
NSUB = 2
LAG = 3
NIT = (NTILE - 1 - LAG) // NSUB
NC = 3
CW = DFF // NC
KA = 256
EPS = 1e-5
NT = (((1,), (1,)), ((), ()))
NN = (((1,), (0,)), ((), ()))
bf16 = jnp.bfloat16
f32 = jnp.float32
u32 = jnp.uint32
QSCALE = (DH ** -0.5) * math.log2(math.e)
L_LO = 2.0 ** -50
L_HI = 2.0 ** 100
O_BIG = 1e30
TORDER = ((0, 8, 1, 2, 4, 5, 6, 7, 3), (0, 8, 1, 2, 3, 4, 5, 6, 7),
          (0, 8, 7, 1, 2, 3, 4, 5, 6), (0, 8, 6, 7, 1, 2, 3, 4, 5))
PROLOGUE = (
    "Q2 W0 V0 r2 Z0 p Z1 Y0 W1 p p Y1 V1 p p p p q q p q q q p L3 q p p p T0 p V2 p W2 q q q "
    "Y2 Z2 q q p q p p p p K3 q q q q p p k3 V3 W3 p Q3 Z3 p p r3 T1 Y3 ")
STEADY = (
    "LA OA q q p q MA p KA kA LB p aA QA q q ZA VA YA q p rA WA q p TA bA cA p 1A p 2A q YB "
    "OB WB KB q p MB 3A ZB q p 0A q 4A q VB TB p kB QB q rB p aB q q q p bB cB p 2B p 1B p 4B "
    "p 0B 3B ")
EPILOGUE = (
    "q q Ta q q O0 O1 M0 p a0 M1 p b0 p c0 q q q q d01 p d00 d03 p p d04 p d02 S0 p a1 O2 Tb "
    "b1 c1 d12 d14 d10 M2 U a2 d13 d11 S1 O3 M3 b2 c2 d23 a3 d21 b3 c3 d24 d30 d31 d20 d22 S2 "
    "d33 d34 d32 ")


def _as_u32(x):
    return pltpu.bitcast(x, u32)


def _as_bf(x):
    return pltpu.bitcast(x, bf16)


def _rows(n, size, count=1):
    if isinstance(n, int):
        return pl.ds(n * size, count * size)
    return pl.ds(pl.multiple_of(n * size, size), count * size)


def _layernorm(x):
    m = jnp.mean(x, axis=-1, keepdims=True)
    xc = x - m
    v = jnp.mean(xc * xc, axis=-1, keepdims=True)
    return xc * lax.rsqrt(v + EPS)


def _quads(y):
    lane = lax.broadcasted_iota(jnp.int32, (y.shape[0], 128), 1)
    out = []
    for g in range(8):
        c0 = (80 * g) // 128
        c1 = (80 * g + 79) // 128
        a = y[:, 128 * c0:128 * c0 + 128]
        if c1 != c0:
            a = jnp.where(lane >= (80 * g) % 128, a, y[:, 128 * c1:128 * c1 + 128])
        out.append(a)
    return out


def _fill_tables(tab):
    lane = lax.broadcasted_iota(jnp.int32, (16, 128), 1)
    row = lax.broadcasted_iota(jnp.int32, (16, 128), 0)
    ones = jnp.uint32(0xFFFFFFFF)
    zero = jnp.uint32(0)
    for h in range(32):
        tab[h] = jnp.where(((lane - (20 * h) % 128) & 127) < 20, ones, zero)
    i = lane & 31
    low = (jnp.where(2 * row <= i, jnp.uint32(0xFFFF), zero)
           | jnp.where(2 * row + 1 <= i, jnp.uint32(0xFFFF0000), zero))
    tab[32] = low
    tab[33] = ~low


def _masks():
    row32 = lax.broadcasted_iota(jnp.int32, (32, 128), 0)
    lane32 = lax.broadcasted_iota(jnp.int32, (32, 128), 1)
    blk = lax.broadcasted_iota(jnp.int32, (16, 128), 1) >> 5
    return dict(tri=row32 <= (lane32 & 31), b0=(blk & 1) == 1, b1=(blk & 2) == 2,
                sub8=lax.broadcasted_iota(jnp.int32, (8, 128), 0) < 4)


def _scores_to_probs(kq, qu, hm, M, tab, true_max, g0):
    tri = M['tri']
    probs = []
    for s in range(4):
        qs = qu[16 * s:16 * s + 16]
        w_t = _as_bf(jnp.concatenate([qs & hm[(p - s) % 4] for p in range(4)], axis=0))
        order = [t for t in TORDER[s] if s + t >= g0]
        lhs = jnp.concatenate([kq[16 * (s + t - g0):16 * (s + t - g0) + 16] for t in order], axis=0)
        st = lax.dot_general(_as_bf(lhs), w_t, NT, preferred_element_type=f32)
        gr = {t: st[32 * i:32 * i + 32] for i, t in enumerate(order)}
        if g0:
            out = {8: _as_u32(jnp.exp2(jnp.where(tri, gr[8], -1e9)).astype(bf16))}
            rest = order[1:]
        else:
            comb = jnp.where(tri, gr[8], gr[0])
            if true_max:
                m = jnp.maximum(jnp.max(comb, axis=0, keepdims=True),
                                jnp.max(st[64:], axis=0, keepdims=True))
                comb = comb - m
                gr = {t: v - m for t, v in gr.items()}
            e = _as_u32(jnp.exp2(comb).astype(bf16))
            out = {0: e & tab[33], 8: e & tab[32]}
            rest = order[2:]
        for t in rest:
            out[t] = _as_u32(jnp.exp2(gr[t]).astype(bf16))
        probs.append(out)

    z = jnp.zeros((16, 128), u32)

    def sel(c, x, y):
        if x is None and y is None:
            return None
        return jnp.where(c, z if x is None else x, z if y is None else y)

    dest = [[] for _ in range(4)]
    for gm in range(g0, 12):
        src = [probs[s].get(gm - s) for s in range(4)]
        t = [sel(M['b0'], src[(i + 1) % 4], src[i]) for i in range(4)]
        for i in range(4):
            d = sel(M['b1'], t[(i + 2) % 4], t[i])
            dest[i].append(z if d is None else d)
    return [_as_bf(jnp.concatenate(dest[(-a) % 4], axis=0)) for a in range(4)]


def _probs_to_out(P, vt, M, bad):
    o = []
    for a in range(4):
        oa = lax.dot_general(vt(a), P[a], NN, preferred_element_type=f32)
        mid = oa[16:24]
        rot = pltpu.roll(mid, 4, 0)
        l = jnp.where(M['sub8'], mid, rot) if a % 2 else jnp.where(M['sub8'], rot, mid)
        r = pl.reciprocal(l, approx=True)
        o3 = oa * jnp.concatenate([r, r, r], axis=0)
        if bad is not None:
            t = o3[0:8] + o3[8:16] + o3[16:24]
            ok = (l >= L_LO) & (l <= L_HI) & (jnp.abs(t) <= O_BIG)
            bad = jnp.where(ok, bad, 1.0)
        if a:
            o3 = pltpu.roll(o3, 128 - 32 * a, 1)
        o.append(o3)
    rows = []
    for m in range(2):
        e, od = o[2 * m], o[2 * m + 1]
        rows += [e[0:16], jnp.where(M['sub8'], e[16:24], od[16:24]), od[0:16]]
    return jnp.concatenate(rows, axis=0), bad


def _kernel(x_hbm, wqkv_hbm, wo_hbm, w1_hbm, w2_hbm, out_hbm,
            x_s, wq_s, wk_s, wv_s, wo_s, w1_s, w2_s, wvt_s, k_s, vt_s, q_s, o_s, out_s, tab,
            ot0, ot1, h0, h1, hid_s, in_sems, out_sems):
    cp = pltpu.make_async_copy
    ot_s = (ot0, ot1)
    h_s = (h0, h1)
    M = {}
    state = dict(bad=jnp.zeros((8, 128), f32))

    def x_copy(n, count, sem):
        r = _rows(n, TT, count)
        return cp(x_hbm.at[r], x_s.at[r], in_sems.at[sem])

    c_x0 = x_copy(0, 3, 0)
    c_wka = cp(wqkv_hbm.at[:, D:D + KA], wk_s.at[:, 0:KA], in_sems.at[1])
    c_wkb = cp(wqkv_hbm.at[:, D + KA:2 * D], wk_s.at[:, KA:D], in_sems.at[2])
    c_wq = cp(wqkv_hbm.at[:, 0:D], wq_s, in_sems.at[3])
    c_x1 = x_copy(3, 1, 4)
    c_wv = cp(wqkv_hbm.at[:, 2 * D:3 * D], wv_s, in_sems.at[4])
    c_wo = cp(wo_hbm, wo_s, in_sems.at[5])
    c_w1 = cp(w1_hbm, w1_s, in_sems.at[5])
    c_w2 = cp(w2_hbm, w2_s, in_sems.at[5])

    def c_xi(it):
        return x_copy(LAG + 1 + NSUB * it, NSUB, 6 + it)

    for c in [c_x0, c_wka, c_wkb, c_wq, c_x1, c_wv, c_wo, c_w1, c_xi(0), c_w2]:
        c.start()
    for it in range(1, NIT):
        c_xi(it).start()

    _fill_tables(tab)

    def pre_tasks(n):
        st = {}

        def ln():
            st['xn'] = _layernorm(x_s[_rows(n, TT), :].astype(f32)).astype(bf16)

        def put(ref_set, y, gs):
            qs = _quads(y)
            for g in gs:
                ref_set(g, qs[g])

        def set_q(g, t):
            q_s[n, g] = t.astype(bf16)

        def set_k(g, t):
            k_s[g, _rows(n + 2, 64), :] = _as_u32(t.astype(bf16))

        def sdot(w, parts):
            if parts == 1:
                return jnp.dot(st['xn'], w, preferred_element_type=f32)
            r = TT // parts
            return jnp.concatenate([jnp.dot(st['xn'][i * r:(i + 1) * r], w, preferred_element_type=f32) for i in range(parts)], axis=0)

        def half(w_s, setter, scale, key, part):
            sp = (2, 4)[part] if (isinstance(n, int) and n == 2 and key == 'k') else 1
            if part == 0:
                y = sdot(w_s[:, 0:KA], sp)
                if scale:
                    y = y * QSCALE
                st[key] = y[:, 128:256]
                put(setter, jnp.concatenate([y, y[:, 0:128], y], axis=1), (0, 1, 2))
            else:
                y = sdot(w_s[:, KA:D], sp)
                if scale:
                    y = y * QSCALE
                put(setter, jnp.concatenate([st[key], st[key], y], axis=1), (3, 4, 5, 6, 7))

        def v(c):
            vt = lax.dot_general(wvt_s[160 * c:160 * c + 160, :], st['xn'], NT, preferred_element_type=f32)
            rows = []
            for m in range(4):
                mid = vt[40 * m + 16:40 * m + 24]
                rows += [vt[40 * m:40 * m + 16], jnp.where(M['sub8'], mid, 1.0),
                         vt[40 * m + 24:40 * m + 40], jnp.where(M['sub8'], 1.0, mid)]
            vt_s[n + 2, 192 * c:192 * c + 192, :] = jnp.concatenate(rows, axis=0)

        return dict(ln=ln, ka=lambda: half(wk_s, set_k, False, 'k', 0), kb=lambda: half(wk_s, set_k, False, 'k', 1),
                    qa=lambda: half(wq_s, set_q, True, 'q', 0), qb=lambda: half(wq_s, set_q, True, 'q', 1),
                    v=[functools.partial(v, c) for c in range(4)])

    pending = {}

    def do_qk(n, g, key, slow=False):
        t0 = max(2 - n, 0) if isinstance(n, int) else 0
        hm = [tab[4 * g + a] for a in range(4)]
        pending[key] = _scores_to_probs(k_s[g, _rows(n + t0, 64, 3 - t0), :], _as_u32(q_s[n, g]),
                                        hm, M, tab, slow, 4 * t0)

    def do_pv(n, g, key, par, slow=False):
        t0 = max(2 - n, 0) if isinstance(n, int) else 0

        def vt(a):
            return jnp.concatenate([vt_s[n + t, _rows(3 * (4 * g + a), 8, 3), :] for t in range(t0, 3)], axis=1)

        o, bad = _probs_to_out(pending.pop(key), vt, M, None if slow else state['bad'])
        if not slow:
            state['bad'] = bad
        ot_s[par][_rows(5 * g, 16, 5), :] = o.astype(bf16)

    def transpose_task(n, par):
        def f():
            o_s[n] = ot_s[par][...].astype(f32).T.astype(bf16)
        return f

    def run(prog, tiles, par0, tasks, started=0):
        units = [(n, g, (i, g)) for i, n in enumerate(tiles) for g in range(8)]
        nq, npv = started, 0
        for tok in prog.split():
            if tok == 'q':
                do_qk(*units[nq])
                nq += 1
            elif tok == 'p':
                do_pv(*units[npv], par=(par0 + npv // 8) % 2)
                npv += 1
            else:
                tasks[tok]()
        assert nq == len(units) and npv == len(units)

    def post_tasks(n, slot):
        st = {'h1': []}
        hs = h_s[slot]

        def proj():
            att = jnp.dot(o_s[n], wo_s[...], preferred_element_type=f32)
            hs[0] = x_s[_rows(n, TT), :].astype(f32) + att

        def ln():
            st['hn'] = _layernorm(hs[0]).astype(bf16)

        def up(c):
            y = jnp.dot(st['hn'], w1_s[:, c * CW:(c + 1) * CW], preferred_element_type=f32)
            st['h1'].append(jnp.maximum(y, 0.0).astype(bf16))

        def down(c):
            cs = slice(c * 128, (c + 1) * 128)
            y = hs[0, :, cs]
            for kc in range(NC):
                y = y + jnp.dot(st['h1'][kc], w2_s[kc * CW:(kc + 1) * CW, cs], preferred_element_type=f32)
            out_s[_rows(n, TT), cs] = y.astype(bf16)

        return dict(proj=proj, ln=ln, up=[functools.partial(up, c) for c in range(NC)],
                    down=[functools.partial(down, c) for c in range(D // 128)])

    def out_copy(n, count):
        r = _rows(n, TT, count)
        return cp(out_s.at[r], out_hbm.at[r], out_sems.at[0])

    def last_copy(c):
        r = _rows(NTILE - 1, TT)
        cs = pl.ds(c * 128, 128)
        return cp(out_s.at[r, cs], out_hbm.at[r, cs], out_sems.at[0])

    M.update(_masks())
    P = [pre_tasks(n) for n in range(LAG + 1)]
    c_x0.wait()
    P[0]['ln']()
    P[1]['ln']()
    c_wka.wait()
    P[2]['ln']()
    for n in range(3):
        P[n]['ka']()
    c_wkb.wait()
    for n in range(3):
        P[n]['kb']()
    c_wq.wait()
    for n in range(2):
        P[n]['qa']()
        P[n]['qb']()
    for g in range(8):
        do_qk(0, g, (0, g))
    c_x1.wait()
    c_wv.wait()
    wvt_s[...] = wv_s[...].astype(f32).T.astype(bf16)
    tasks = dict(T0=transpose_task(0, 0), T1=transpose_task(1, 1), L3=P[3]['ln'], K3=P[3]['ka'], k3=P[3]['kb'],
                 Q2=P[2]['qa'], r2=P[2]['qb'], Q3=P[3]['qa'], r3=P[3]['qb'])
    for n in range(4):
        for c in range(4):
            tasks['VWYZ'[c] + str(n)] = P[n]['v'][c]
    run(PROLOGUE, [0, 1, 2], 0, tasks, started=8)
    c_wo.wait()
    c_w1.wait()
    c_w2.wait()

    def tile_tasks(n, par):
        F = post_tasks(n - LAG, par)
        N = pre_tasks(n + 1)
        T = dict(O=F['proj'], L=N['ln'], K=N['ka'], k=N['kb'], M=F['ln'], T=transpose_task(n - 1, par), V=N['v'][0], W=N['v'][1],
                 Y=N['v'][2], Z=N['v'][3], Q=N['qa'], r=N['qb'],
                 a=F['up'][0], b=F['up'][1], c=F['up'][2])
        for i in range(5):
            T[str(i)] = F['down'][i]
        return T

    def loop_body(it, bad):
        state['bad'] = bad
        M.update(_masks())
        n0 = LAG + it * NSUB
        c_xi(it).wait()
        TA, TB = tile_tasks(n0, 0), tile_tasks(n0 + 1, 1)
        tasks = {k + 'A': v for k, v in TA.items()}
        tasks.update({k + 'B': v for k, v in TB.items()})
        run(STEADY, [n0, n0 + 1], 1, tasks)
        out_copy(n0 - LAG, NSUB).start()
        return state['bad']

    state['bad'] = lax.fori_loop(0, NIT, loop_body, state['bad'])

    M.update(_masks())
    n0 = NTILE - 1 - LAG
    F = [post_tasks(n0 + i, i % 2) for i in range(LAG + 1)]

    def send(i):
        return lambda: out_copy(n0 + i, 1).start()

    tasks = dict(Ta=transpose_task(NTILE - 2, 0), Tb=transpose_task(NTILE - 1, 1))
    flag = {}
    tasks['U'] = lambda: flag.update(u=jnp.max(state['bad']))
    for i in range(LAG + 1):
        tasks['O%d' % i] = F[i]['proj']
        tasks['M%d' % i] = F[i]['ln']
        for c in range(NC):
            tasks['abc'[c] + str(i)] = F[i]['up'][c]
        for c in range(5):
            tasks['d%d%d' % (i, c)] = F[i]['down'][c]
        tasks['S%d' % i] = send(i)
    for c in range(5):
        tasks['d3%d' % c] = (lambda c: lambda: (F[LAG]['down'][c](), last_copy(c).start()))(c)
    run(EPILOGUE, [NTILE - 1], 1, tasks)
    unsafe = flag['u']

    for it in range(NIT):
        out_copy(it * NSUB, NSUB).wait()
    for i in range(LAG):
        out_copy(n0 + i, 1).wait()
    for c in range(D // 128):
        last_copy(c).wait()

    @pl.when(unsafe > 0.0)
    def _():
        vt_s[0:2] = jnp.zeros((2,) + vt_s.shape[1:], f32)
        for g in range(8):
            k0 = k_s[g, 128:129, :] & jnp.uint32(0xFFFF)
            k_s[g, 0:128, :] = jnp.broadcast_to(k0 | (k0 << 16), (128, 128))

        def slow_tile(n, carry):
            M.update(_masks())

            def slow_quad(g, c):
                do_qk(n, g, 'slow', True)
                do_pv(n, g, 'slow', 0, True)
                return c

            lax.fori_loop(0, 8, slow_quad, 0)
            o = ot0[...].astype(f32).T.astype(bf16)
            h0[0] = x_s[_rows(n, TT), :].astype(f32) + jnp.dot(o, wo_s[...], preferred_element_type=f32)
            hn = _layernorm(h0[0]).astype(bf16)

            def slow_up(c, c2):
                cs = _rows(c, 128)
                y = jnp.dot(hn, w1_s[:, cs], preferred_element_type=f32)
                hid_s[:, cs] = jnp.maximum(y, 0.0).astype(bf16)
                return c2

            lax.fori_loop(0, DFF // 128, slow_up, 0)

            def slow_down(c, c2):
                cs = _rows(c, 128)
                y = h0[0, :, cs] + jnp.dot(hid_s[...], w2_s[:, cs], preferred_element_type=f32)
                out_s[_rows(n, TT), cs] = y.astype(bf16)
                return c2

            lax.fori_loop(0, D // 128, slow_down, 0)
            return carry

        lax.fori_loop(0, NTILE, slow_tile, 0)
        c = cp(out_s, out_hbm, out_sems.at[0])
        c.start()
        c.wait()


@jax.jit
def pallas_sequential_preLN__sliding_block__dense_activation_relu__prompt_kernel(
    A_x: jax.Array,
    A_wqkv: jax.Array,
    A_wo: jax.Array,
    B_x: jax.Array,
    B_w1: jax.Array,
    B_w2: jax.Array,
):
    del B_x
    V = pltpu.VMEM
    hbm = pl.BlockSpec(memory_space=pl.ANY)
    out = pl.pallas_call(
        _kernel,
        in_specs=[hbm] * 5,
        out_specs=hbm,
        out_shape=jax.ShapeDtypeStruct((S, D), bf16),
        scratch_shapes=[
            V((S, D), bf16),
            V((D, D), bf16), V((D, D), bf16), V((D, D), bf16), V((D, D), bf16),
            V((D, DFF), bf16), V((DFF, D), bf16),
            V((D, D), bf16),
            V((8, (S + W) // 2, 128), u32),
            V((NTILE + 2, 768, 128), f32),
            V((NTILE, 8, TT, 128), bf16),
            V((NTILE, TT, D), bf16),
            V((S, D), bf16),
            V((34, 16, 128), u32),
            V((D, TT), bf16), V((D, TT), bf16),
            V((1, TT, D), f32), V((1, TT, D), f32),
            V((TT, DFF), bf16),
            pltpu.SemaphoreType.DMA((6 + NIT,)),
            pltpu.SemaphoreType.DMA((1,)),
        ],
        compiler_params=pltpu.CompilerParams(vmem_limit_bytes=100 * 1024 * 1024),
    )(A_x.reshape(S, D), A_wqkv, A_wo, B_w1, B_w2)
    return out.reshape(1, S, D)
```
